```python
import jax
import jax.numpy as jnp

def _softmax(x, axis=-1):
    return jax.nn.softmax(x, axis=axis)
def _gelu(x):
    return jax.nn.gelu(x, approximate=True)
def _silu(x):
    return jax.nn.silu(x)
def _sigmoid(x):
    return jax.nn.sigmoid(x)
def _layernorm(x, axis=-1, eps=1e-5):
    m = jnp.mean(x, axis=axis, keepdims=True)
    v = jnp.var(x, axis=axis, keepdims=True)
    return (x - m) / jnp.sqrt(v + eps)
def _scatter_add(tgt, idx, src, axis=0):
    return tgt.at[idx].add(src)
def _segment_sum(src, seg, n):
    return jax.ops.segment_sum(src, seg, n)
class _Rng:
    def __init__(self, key):
        self._k = key
    def _next(self):
        self._k, sub = jax.random.split(self._k)
        return sub
    def normal(self, shape):
        return jax.random.normal(self._next(), shape, dtype=jnp.bfloat16)
    def randint(self, lo, hi, shape):
        return jax.random.randint(self._next(), shape, lo, hi, dtype=jnp.int32)
    def uniform(self, shape, lo=0.0, hi=1.0):
        return jax.random.uniform(self._next(), shape, jnp.bfloat16, lo, hi)
    def permutation(self, n):
        return jax.random.permutation(self._next(), n)


kernel_name = 'standalone__modern_conv_block_replknet__vision'

def setup_inputs():
    _rng = _Rng(jax.random.key(int.from_bytes(__import__("os").urandom(4), "little")))
    _w = (lambda a: (lambda t: t.astype(jnp.bfloat16) if jnp.issubdtype(t.dtype, jnp.floating) else t)(jnp.asarray(a)))
    H = W = 512
    C = 96
    K = 3
    return {
        "x": _w((lambda *s: _rng.normal(s) * 0.05)(1, H, W, C)),
        "dw_large": _w((lambda *s: _rng.normal(s) * 0.05)(K, K, C) * (1.0 / K)),
        "dw_small": _w((lambda *s: _rng.normal(s) * 0.05)(5, 5, C) * 0.2),
        "w1": _w((lambda *s: _rng.normal(s) * 0.05)(C, 4 * C) * (C ** -0.5)),
        "w2": _w((lambda *s: _rng.normal(s) * 0.05)(4 * C, C) * ((4 * C) ** -0.5)),
    }

def reference(x, dw_large, dw_small, w1, w2):
    B, H, W, C = x.shape
    Kl = dw_large.shape[0]
    pl = (Kl - 1) // 2
    xpl = jnp.pad(x, ((0,0),(pl,pl),(pl,pl),(0,0)))
    out = jnp.zeros_like(x)
    for i in range(Kl):
        for j in range(Kl):
            out = out + xpl[:, i:i+H, j:j+W, :] * dw_large[i, j][None, None, None, :]
    Ks = dw_small.shape[0]
    ps = (Ks - 1) // 2
    xps = jnp.pad(x, ((0,0),(ps,ps),(ps,ps),(0,0)))
    for i in range(Ks):
        for j in range(Ks):
            out = out + xps[:, i:i+H, j:j+W, :] * dw_small[i, j][None, None, None, :]
    h = _layernorm(out, axis=-1)
    h = _gelu(jnp.einsum('bhwc,ce->bhwe', h, w1))
    h = jnp.einsum('bhwe,ec->bhwc', h, w2)
    return x + h
```

```python
import jax
import jax.numpy as jnp
import jax.experimental.pallas as pl
import jax.experimental.pallas.tpu as pltpu

TH = 16
F32 = jnp.float32
BF = jnp.bfloat16


def _kernel(xp_ref, x_ref, xn_ref, dl_ref, ds_ref, w1_ref, w2_ref, o_ref,
            xs, wb, ln):
    C, W = x_ref.shape[1], x_ref.shape[2]
    i = pl.program_id(0)
    n = pl.num_programs(0)

    @pl.when(i == 0)
    def _():
        for a in range(5):
            for b in range(5):
                v = ds_ref[:, a * 5 + b:a * 5 + b + 1].astype(F32)
                if 1 <= a <= 3 and 1 <= b <= 3:
                    k = (a - 1) * 3 + b - 1
                    v = v + dl_ref[:, k:k + 1].astype(F32)
                wb[a * 5 + b] = jnp.broadcast_to(v, (C, 128))

    xs[0:2] = jnp.where(i > 0, xp_ref[...].astype(F32), 0.0)
    xs[TH + 2:TH + 4] = jnp.where(i < n - 1, xn_ref[...].astype(F32), 0.0)

    def cp(r, c):
        xs[r + 2] = x_ref[r].astype(F32)
        return c
    jax.lax.fori_loop(0, TH, cp, 0)

    NV = W // 128
    lane = jax.lax.broadcasted_iota(jnp.int32, (8, 128), 1)

    def conv_ln(r):
        rows = []
        for g in range(C // 8):
            cs = slice(g * 8, g * 8 + 8)
            xv = [[xs[r + a, cs, k * 128:(k + 1) * 128] for k in range(NV)]
                  for a in range(5)]
            acc = None
            for b in (2, 0, 1, 3, 4):
                p = []
                for k in range(NV):
                    t = xv[0][k] * wb[b, cs, :]
                    for a in range(1, 5):
                        t = t + xv[a][k] * wb[a * 5 + b, cs, :]
                    p.append(t)
                s = 2 - b
                if s == 0:
                    acc = p
                    continue
                rr = [pltpu.roll(t, s % 128, 1) for t in p]
                for k in range(NV):
                    if s > 0:
                        o = rr[k - 1] if k > 0 else 0.0
                        v = jnp.where(lane < s, o, rr[k])
                    else:
                        o = rr[k + 1] if k < NV - 1 else 0.0
                        v = jnp.where(lane >= 128 + s, o, rr[k])
                    acc[k] = acc[k] + v
            rows.append(jnp.concatenate(acc, axis=1))
        y = jnp.concatenate(rows, axis=0)
        m = jnp.sum(y, axis=0, keepdims=True) * (1.0 / C)
        d = y - m
        v = jnp.sum(d * d, axis=0, keepdims=True) * (1.0 / C)
        return (d * jax.lax.rsqrt(v + 1e-5)).astype(BF)

    def ffn(r, l):
        h = jnp.dot(w1_ref[...], l, preferred_element_type=F32)
        u = h * (h * h * 0.035677408136300125 + 0.7978845608028654)
        hh = 0.5 * h
        g = (hh + hh * jnp.tanh(u)).astype(BF)
        o = jnp.dot(w2_ref[...], g, preferred_element_type=F32)
        o_ref[r] = (xs[r + 2] + o).astype(BF)

    ln[...] = conv_ln(0)

    def body(r, c):
        l = ln[...]
        ln[...] = conv_ln(r)
        ffn(r - 1, l)
        return c
    jax.lax.fori_loop(1, TH, body, 0)
    ffn(TH - 1, ln[...])


@jax.jit
def pallas_standalone__modern_conv_block_replknet__vision_kernel(
    x, dw_large, dw_small, w1, w2):
    _, H, W, C = x.shape
    xt = x.reshape(H, W, C).transpose(0, 2, 1)
    nb = H // TH
    hb = TH // 2
    full = lambda s: pl.BlockSpec(s, lambda i: (0,) * len(s))
    out = pl.pallas_call(
        _kernel,
        grid=(nb,),
        in_specs=[
            pl.BlockSpec((2, C, W), lambda i: (jnp.maximum(i * hb - 1, 0), 0, 0)),
            pl.BlockSpec((TH, C, W), lambda i: (i, 0, 0)),
            pl.BlockSpec((2, C, W), lambda i: (jnp.minimum(i * hb + hb, H // 2 - 1), 0, 0)),
            full((C, 9)), full((C, 25)), full((4 * C, C)), full((C, 4 * C)),
        ],
        out_specs=pl.BlockSpec((TH, C, W), lambda i: (i, 0, 0)),
        out_shape=jax.ShapeDtypeStruct((H, C, W), x.dtype),
        scratch_shapes=[pltpu.VMEM((TH + 4, C, W), F32),
                        pltpu.VMEM((25, C, 128), F32),
                        pltpu.VMEM((C, W), BF)],
        compiler_params=pltpu.CompilerParams(
            dimension_semantics=("arbitrary",),
            vmem_limit_bytes=64 * 1024 * 1024),
    )(xt, xt, xt, dw_large.reshape(9, C).T, dw_small.reshape(25, C).T, w1.T, w2.T)
    return out.transpose(0, 2, 1).reshape(1, H, W, C)
```

```python
import jax
import jax.numpy as jnp
import jax.experimental.pallas as pl
import jax.experimental.pallas.tpu as pltpu

TH = 32
S = 0.035677408136300125 ** (1.0 / 3.0)
F32 = jnp.float32
BF = jnp.bfloat16


def _kernel(xp_ref, x_ref, xn_ref, dl_ref, ds_ref, w1_ref, w2_ref, o_ref,
            xs, wb, ln, w2h):
    C, W = x_ref.shape[1], x_ref.shape[2]
    i = pl.program_id(0)
    n = pl.num_programs(0)

    @pl.when(i == 0)
    def _():
        w2h[...] = (w2_ref[...].astype(F32) * (0.5 / S)).astype(BF)
        for a in range(5):
            for b in range(5):
                v = ds_ref[:, a * 5 + b:a * 5 + b + 1].astype(F32)
                if 1 <= a <= 3 and 1 <= b <= 3:
                    k = (a - 1) * 3 + b - 1
                    v = v + dl_ref[:, k:k + 1].astype(F32)
                wb[a * 5 + b] = jnp.broadcast_to(v, (C, 128))

    xs[0:2] = jnp.where(i > 0, xp_ref[...].astype(F32), 0.0)
    xs[TH + 2:TH + 4] = jnp.where(i < n - 1, xn_ref[...].astype(F32), 0.0)

    xs[2:5] = x_ref[0:3].astype(F32)

    NV = W // 128
    lane = jax.lax.broadcasted_iota(jnp.int32, (8, 128), 1)

    def conv_ln(r, par, hook=None):
        for g in range(C // 8):
            cs = slice(g * 8, g * 8 + 8)
            xv = [[xs[r + a, cs, k * 128:(k + 1) * 128] for k in range(NV)]
                  for a in range(5)]
            acc = None
            for b in (2, 0, 1, 3, 4):
                p = []
                for k in range(NV):
                    t = xv[0][k] * wb[b, cs, :]
                    for a in range(1, 5):
                        t = t + xv[a][k] * wb[a * 5 + b, cs, :]
                    p.append(t)
                s = 2 - b
                if s == 0:
                    acc = p
                    continue
                rr = [pltpu.roll(t, s % 128, 1) for t in p]
                for k in range(NV):
                    if s > 0:
                        o = rr[k - 1] if k > 0 else 0.0
                        v = jnp.where(lane < s, o, rr[k])
                    else:
                        o = rr[k + 1] if k < NV - 1 else 0.0
                        v = jnp.where(lane >= 128 + s, o, rr[k])
                    acc[k] = acc[k] + v
            for k in range(NV):
                ln[par, cs, k * 128:(k + 1) * 128] = acc[k]
            if hook is not None and g % GS == 0:
                hook(g // GS)

    NC = 1
    GS = 12 // NC
    CW = W // NC

    def ffn(r, k, par):
        ws = slice(k * CW, (k + 1) * CW)
        y = ln[par, :, ws]
        m = jnp.sum(y, axis=0, keepdims=True) * (1.0 / C)
        d = y - m
        v = jnp.sum(d * d, axis=0, keepdims=True) * (1.0 / C)
        l = (d * (jax.lax.rsqrt(v + 1e-5) * S)).astype(BF)
        h = jnp.dot(w1_ref[...], l, preferred_element_type=F32)
        u = h * (h * h + 0.7978845608028654 / S)
        g = (h + h * jnp.tanh(u)).astype(BF)
        o = jnp.dot(w2h[...], g, preferred_element_type=F32)
        o_ref[r, :, ws] = (xs[r + 2, :, ws] + o).astype(BF)

    conv_ln(0, 0)
    xs[5] = x_ref[3].astype(F32)

    def row(r, par):
        conv_ln(r, par, lambda k: ffn(r - 1, k, 1 - par))
        q = jnp.minimum(r + 3, TH - 1)
        xs[q + 2] = x_ref[q].astype(F32)

    def body(j, c):
        row(2 * j, 0)
        row(2 * j + 1, 1)
        return c
    row(1, 1)
    jax.lax.fori_loop(1, TH // 2, body, 0)
    for k in range(NC):
        ffn(TH - 1, k, 1)


@jax.jit
def pallas_standalone__modern_conv_block_replknet__vision_kernel(
    x, dw_large, dw_small, w1, w2):
    _, H, W, C = x.shape
    xt = x.reshape(H, W, C).transpose(0, 2, 1)
    nb = H // TH
    hb = TH // 2
    full = lambda s: pl.BlockSpec(s, lambda i: (0,) * len(s))
    out = pl.pallas_call(
        _kernel,
        grid=(nb,),
        in_specs=[
            pl.BlockSpec((2, C, W), lambda i: (jnp.maximum(i * hb - 1, 0), 0, 0)),
            pl.BlockSpec((TH, C, W), lambda i: (i, 0, 0)),
            pl.BlockSpec((2, C, W), lambda i: (jnp.minimum(i * hb + hb, H // 2 - 1), 0, 0)),
            full((C, 9)), full((C, 25)), full((4 * C, C)), full((C, 4 * C)),
        ],
        out_specs=pl.BlockSpec((TH, C, W), lambda i: (i, 0, 0)),
        out_shape=jax.ShapeDtypeStruct((H, C, W), x.dtype),
        scratch_shapes=[pltpu.VMEM((TH + 4, C, W), F32),
                        pltpu.VMEM((25, C, 128), F32),
                        pltpu.VMEM((2, C, W), F32),
                        pltpu.VMEM((C, 4 * C), BF)],
        compiler_params=pltpu.CompilerParams(
            dimension_semantics=("arbitrary",),
            flags={"XLA_TPU_FORCE_LP_LLO_SCHEDULER": True},
            vmem_limit_bytes=64 * 1024 * 1024),
    )(xt, xt, xt, dw_large.reshape(9, C).T, dw_small.reshape(25, C).T, w1.T, w2.T)
    return out.transpose(0, 2, 1).reshape(1, H, W, C)
```

```python
import jax
import jax.numpy as jnp
import jax.experimental.pallas as pl
import jax.experimental.pallas.tpu as pltpu

TH = 32
S = 0.035677408136300125 ** (1.0 / 3.0)
F32 = jnp.float32
BF = jnp.bfloat16


HN = 8


def _kernel(x_ref, xn_ref, dl_ref, ds_ref, w1_ref, w2_ref, o_ref,
            xs, wb, yb, lb, gb, w2h):
    C, W = x_ref.shape[1], x_ref.shape[2]
    i = pl.program_id(0)
    n = pl.num_programs(0)
    NV = W // 128
    NG = C // 8
    lane = jax.lax.broadcasted_iota(jnp.int32, (8, 128), 1)

    xs[2:8] = x_ref[0:6].astype(F32)
    xs[TH + 2:TH + 8] = jnp.where(i < n - 1, xn_ref[0:6].astype(F32), 0.0)

    def conv(r, g):
        cs = slice(g * 8, g * 8 + 8)
        xv = [[xs[r + a, cs, k * 128:(k + 1) * 128] for k in range(NV)]
              for a in range(5)]
        acc = None
        for b in (2, 0, 1, 3, 4):
            p = []
            for k in range(NV):
                t = xv[0][k] * wb[b, cs, :]
                for a in range(1, 5):
                    t = t + xv[a][k] * wb[a * 5 + b, cs, :]
                p.append(t)
            s = 2 - b
            if s == 0:
                acc = p
                continue
            rr = [pltpu.roll(t, s % 128, 1) for t in p]
            for k in range(NV):
                if s > 0:
                    o = rr[k - 1] if k > 0 else 0.0
                    v = jnp.where(lane < s, o, rr[k])
                else:
                    o = rr[k + 1] if k < NV - 1 else 0.0
                    v = jnp.where(lane >= 128 + s, o, rr[k])
                acc[k] = acc[k] + v
        for k in range(NV):
            yb[cs, k * 128:(k + 1) * 128] = acc[k]

    def norm():
        y = yb[...]
        m = jnp.sum(y, axis=0, keepdims=True) * (1.0 / C)
        d = y - m
        v = jnp.sum(d * d, axis=0, keepdims=True) * (1.0 / C)
        lb[...] = (d * (jax.lax.rsqrt(v + 1e-5) * S)).astype(BF)

    def up(ws):
        h = jnp.dot(w1_ref[...], lb[:, ws], preferred_element_type=F32)
        u = h * (h * h + 0.7978845608028654 / S)
        gb[:, ws] = (h + h * jnp.tanh(u)).astype(BF)

    def down(r, ws):
        o = jnp.dot(w2h[...], gb[:, ws], preferred_element_type=F32)
        o_ref[r, :, ws] = (xs[r + 2, :, ws] + o).astype(BF)

    @pl.when(i == 0)
    def _():
        w2h[...] = (w2_ref[...].astype(F32) * (0.5 / S)).astype(BF)
        for a in range(5):
            for b in range(5):
                v = ds_ref[:, a * 5 + b:a * 5 + b + 1].astype(F32)
                if 1 <= a <= 3 and 1 <= b <= 3:
                    k = (a - 1) * 3 + b - 1
                    v = v + dl_ref[:, k:k + 1].astype(F32)
                wb[a * 5 + b] = jnp.broadcast_to(v, (C, 128))
        xs[0:2] = jnp.zeros((2, C, W), F32)
        yb[...] = jnp.zeros(yb.shape, F32)
        lb[...] = jnp.zeros(lb.shape, BF)

        def pro(r, c):
            up(slice(None))
            norm()
            for g in range(NG):
                conv(r, g)
            return c
        jax.lax.fori_loop(0, 3, pro, 0)

    MODE = 0

    def body(t, c):
        if MODE == 0:
            down(t, slice(None))
            up(slice(None))
            norm()
            for g in range(NG):
                conv(t + 3, g)
        else:
            y = yb[...]
            cw = W // MODE
            for k in range(MODE):
                ws = slice(k * cw, (k + 1) * cw)
                down(t, ws)
                up(ws)
            norm()
            for g in range(NG):
                conv(t + 3, g)
        q = jnp.minimum(t + 6, TH - 1)
        xs[q + 2] = x_ref[q].astype(F32)
        return c
    jax.lax.fori_loop(0, TH, body, 0)


@jax.jit
def pallas_standalone__modern_conv_block_replknet__vision_kernel(
    x, dw_large, dw_small, w1, w2):
    _, H, W, C = x.shape
    xt = x.reshape(H, W, C).transpose(0, 2, 1)
    nb = H // TH
    hb = TH // HN
    full = lambda s: pl.BlockSpec(s, lambda i: (0,) * len(s))
    out = pl.pallas_call(
        _kernel,
        grid=(nb,),
        in_specs=[
            pl.BlockSpec((TH, C, W), lambda i: (i, 0, 0)),
            pl.BlockSpec((HN, C, W), lambda i: (jnp.minimum(i * hb + hb, H // HN - 1), 0, 0)),
            full((C, 9)), full((C, 25)), full((4 * C, C)), full((C, 4 * C)),
        ],
        out_specs=pl.BlockSpec((TH, C, W), lambda i: (i, 0, 0)),
        out_shape=jax.ShapeDtypeStruct((H, C, W), x.dtype),
        scratch_shapes=[pltpu.VMEM((TH + 8, C, W), F32),
                        pltpu.VMEM((25, C, 128), F32),
                        pltpu.VMEM((C, W), F32),
                        pltpu.VMEM((C, W), BF),
                        pltpu.VMEM((4 * C, W), BF),
                        pltpu.VMEM((C, 4 * C), BF)],
        compiler_params=pltpu.CompilerParams(
            dimension_semantics=("arbitrary",),
            vmem_limit_bytes=64 * 1024 * 1024),
    )(xt, xt, dw_large.reshape(9, C).T, dw_small.reshape(25, C).T, w1.T, w2.T)
    return out.transpose(0, 2, 1).reshape(1, H, W, C)
```
